```python
import jax
import jax.numpy as jnp

def _softmax(x, axis=-1):
    return jax.nn.softmax(x, axis=axis)
def _gelu(x):
    return jax.nn.gelu(x, approximate=True)
def _silu(x):
    return jax.nn.silu(x)
def _sigmoid(x):
    return jax.nn.sigmoid(x)
def _layernorm(x, axis=-1, eps=1e-5):
    m = jnp.mean(x, axis=axis, keepdims=True)
    v = jnp.var(x, axis=axis, keepdims=True)
    return (x - m) / jnp.sqrt(v + eps)
def _scatter_add(tgt, idx, src, axis=0):
    return tgt.at[idx].add(src)
def _segment_sum(src, seg, n):
    return jax.ops.segment_sum(src, seg, n)
class _Rng:
    def __init__(self, key):
        self._k = key
    def _next(self):
        self._k, sub = jax.random.split(self._k)
        return sub
    def normal(self, shape):
        return jax.random.normal(self._next(), shape, dtype=jnp.bfloat16)
    def randint(self, lo, hi, shape):
        return jax.random.randint(self._next(), shape, lo, hi, dtype=jnp.int32)
    def uniform(self, shape, lo=0.0, hi=1.0):
        return jax.random.uniform(self._next(), shape, jnp.bfloat16, lo, hi)
    def permutation(self, n):
        return jax.random.permutation(self._next(), n)


kernel_name = 'standalone__seq2seq_rnn_t_joint__speech'

def _fwd_setup_inputs():
    _rng = _Rng(jax.random.key(int.from_bytes(__import__("os").urandom(4), "little")))
    _w = (lambda a: (lambda t: t.astype(jnp.bfloat16) if jnp.issubdtype(t.dtype, jnp.floating) else t)(jnp.asarray(a)))
    B, T, D, K = 2, 4000, 256, 3
    U = 8
    sc = (1.0 / (K * D)) ** 0.5
    sd = (1.0 / D) ** 0.5
    return {
        "x": _w((lambda *s: _rng.normal(s) * 0.05)(B, T, D) * 0.5),
        "w1": _w((lambda *s: _rng.normal(s) * 0.05)(K, D, D) * sc),
        "w2": _w((lambda *s: _rng.normal(s) * 0.05)(K, D, D) * sc),
        "g": _w((lambda *s: _rng.normal(s) * 0.05)(B, U, D) * 0.5),
        "w_f": _w((lambda *s: _rng.normal(s) * 0.05)(D, D) * sd),
        "w_g": _w((lambda *s: _rng.normal(s) * 0.05)(D, D) * sd),
        "w_o": _w((lambda *s: _rng.normal(s) * 0.05)(D, D) * sd),
    }

def _fwd_reference(x, w1, w2, g, w_f, w_g, w_o):
    B, T, D = x.shape
    K = w1.shape[0]
    pad = K // 2
    xp = jnp.pad(x, ((0,0),(pad,pad),(0,0)))
    h = jnp.zeros_like(x)
    for i in range(K):
        h = h + jnp.einsum("btc,cd->btd", xp[:, i:i+T, :], w1[i])
    h = _gelu(h)[:, ::2, :]
    T1 = h.shape[1]
    hp = jnp.pad(h, ((0,0),(pad,pad),(0,0)))
    f = jnp.zeros_like(h)
    for i in range(K):
        f = f + jnp.einsum("btc,cd->btd", hp[:, i:i+T1, :], w2[i])
    f = _gelu(f)[:, ::2, :]
    fe = jnp.einsum("btd,de->bte", f, w_f)
    ge = jnp.einsum("bud,de->bue", g, w_g)
    j = jnp.tanh(fe[:, :, None, :] + ge[:, None, :, :])
    return jnp.einsum("btud,dv->btuv", j, w_o)


def setup_inputs():
    _inp = _fwd_setup_inputs()
    _gk = jax.random.fold_in(jax.random.key(int.from_bytes(__import__("os").urandom(4), "little")), 2**31 - 1)
    _shapes = [[2, 1000, 8, 256]]
    _dtypes = ['bfloat16']
    _gks = jax.random.split(_gk, len(_shapes))
    _gs = [jax.random.normal(k, s, dtype=jnp.dtype(d)) * 0.05 for k, s, d in zip(_gks, _shapes, _dtypes)]
    _inp["grad_out"] = _gs[0]
    return _inp

def reference(x, w1, w2, g, w_f, w_g, w_o, grad_out):
    _const = dict()
    def _f(*_d):
        return _fwd_reference(**{'x': _d[0], 'w1': _d[1], 'w2': _d[2], 'g': _d[3], 'w_f': _d[4], 'w_g': _d[5], 'w_o': _d[6], **_const})
    _out, _vjp = jax.vjp(_f, x, w1, w2, g, w_f, w_g, w_o)
    _grads = _vjp(grad_out)
    _out0 = jnp.asarray(_out)
    return (_out0, *[jnp.asarray(_g) for _g in _grads])
```

```python
import functools
import jax
import jax.numpy as jnp
from jax.experimental import pallas as pl
from jax.experimental.pallas import tpu as pltpu

F32 = jnp.float32
BF16 = jnp.bfloat16
U32 = jnp.uint32
U16 = jnp.uint16
L = 128

_C = 0.7978845608028654
_K = 0.044715


def _gelu_and_grad(x):
    x2 = x * x
    t = jnp.tanh(x * (_C + (_C * _K) * x2))
    p = 0.5 + 0.5 * t
    g = x * p
    gp = p + g * (1.0 - p) * (2.0 * _C + (6.0 * _C * _K) * x2)
    return g, gp


def _lo(w):
    return pltpu.bitcast(w << 16, F32)


def _hi(w):
    return pltpu.bitcast(w & jnp.uint32(0xFFFF0000), F32)


def _lo16(w):
    return pltpu.bitcast(w.astype(U16), BF16)


def _hi16(w):
    return pltpu.bitcast((w >> 16).astype(U16), BF16)


def _words(a_bf16):
    return pltpu.bitcast(a_bf16, U32)


def _bf(a):
    return a.astype(BF16)


def _nn(a, b):
    return jnp.dot(a, b, preferred_element_type=F32)


def _nt(a, b):
    return jax.lax.dot_general(a, b, (((1,), (1,)), ((), ())), preferred_element_type=F32)


def _tn(a, b):
    return jax.lax.dot_general(a, b, (((0,), (0,)), ((), ())), preferred_element_type=F32)


def _il(a, b):
    return pltpu.bitcast(pltpu.pack_elementwise([a, b], packed_dtype=BF16), BF16)


def _shift_down(a, prev8):
    ext = jnp.concatenate([prev8, a], axis=0)
    return pltpu.roll(ext, 1, 0)[8:]


def _shift_up(a, next8):
    n = a.shape[0]
    ext = jnp.concatenate([a, next8], axis=0)
    return pltpu.roll(ext, n + 7, 0)[:n]


def _ld(ref, r0, r1, c0=0, c1=None):
    c1 = ref.shape[0] if c1 is None else c1
    parts = [pltpu.bitcast(ref[c, r0 // 2:r1 // 2, :], BF16) for c in range(c0, c1)]
    return parts[0] if len(parts) == 1 else jnp.concatenate(parts, axis=1)


def _ldw(ref, r0, r1):
    return jnp.concatenate([ref[c, r0 // 2:r1 // 2, :] for c in range(ref.shape[0])], axis=1)


def _st(ref, r0, val, c0=0):
    n = val.shape[0]
    w = pltpu.bitcast(val, U32)
    for c in range(val.shape[1] // L):
        ref[c0 + c, r0 // 2:(r0 + n) // 2, :] = w[:, c * L:(c + 1) * L]


def _rowsum8(v):
    s = jax.lax.broadcasted_iota(jnp.int32, v[0].shape, 0)

    def comb(a, b, m, k):
        p = jnp.where(m, a, b)
        q = jnp.where(m, b, a)
        return p + pltpu.roll(q, 8 - k, 0)

    m1 = lambda j: ((s + (8 - j)) & 4) == 0
    m2 = lambda j: ((s + (8 - j)) & 2) == 0
    ab = comb(v[0], v[4], m1(0), 4)
    cd = comb(v[2], v[6], m1(2), 4)
    ef = comb(v[1], v[5], m1(1), 4)
    gh = comb(v[3], v[7], m1(3), 4)
    abcd = comb(ab, cd, m2(0), 2)
    efgh = comb(ef, gh, m2(1), 2)
    return comb(abcd, efgh, (s & 1) == 0, 1)


def _tree_sum(v):
    v = list(v)
    while len(v) > 1:
        v = [v[i] + v[i + 1] if i + 1 < len(v) else v[i] for i in range(0, len(v), 2)]
    return v[0]


def _chunks(total, size):
    if isinstance(size, (tuple, list)):
        out, s = [], 0
        for n in size:
            out.append((s, n))
            s += n
        assert s == total, (size, total)
        return out
    out = []
    s = 0
    while s < total:
        n = min(size, total - s)
        out.append((s, n))
        s += n
    return out


def make_kernel(B, T, D, U, NB, RC1, QC2, QCB, CT, X_PARTS, GO_PARTS):
    TF = T // 4
    NQ = -(-(TF // 2) // 8) * 8
    NQP = -(-NQ // 16) * 16
    NR = 2 * NQ
    XP = 4 * NR
    H = D // L

    sem_ids = {}

    def sid(name):
        return sem_ids.setdefault(name, len(sem_ids))

    def kernel(x_hbm, go_hbm, g_hbm, w1_hbm, w2_hbm, wf_hbm, wg_hbm, wo_hbm,
               out_hbm, dx_hbm, dw1_hbm, dw2_hbm, dg_hbm, dwf_hbm, dwg_hbm, dwo_hbm,
               x_s, go_s, out_s, dx_s, w1_s, w2_s, wf_s, wg_s, wo_s, g_s,
               w1_p, w2_p, wf_p, wg_p, wo_p, ws1_s, ws2_s,
               o_dw1, o_dw2, o_dwf, o_dwg, o_dwo, o_dg,
               a_dw1, a_dw2, a_dwf, a_dwg, a_dwo,
               xa_s, xb_s, x1_s, gpe_s, gpo_s, ha_s, hb_s, h1_s, gp2_s, fb_s, fe_s, dfe_s,
               de_s, do_s, da_s, db_s, ds_s,
               sems):
        def cp(src, dst, name):
            return pltpu.make_async_copy(src, dst, sems.at[sid(name)])

        def start(cs):
            for c in cs:
                c.start()

        def wait(cs):
            for c in cs:
                c.wait()

        def rows_cp(src, dst, lo, n, name):
            return [cp(src.at[pl.ds(lo, n)], dst.at[pl.ds(lo, n)], name)]

        x0_cp = [rows_cp(x_hbm.at[0], x_s.at[0], lo, hi - lo, ("x0", k)) for k, (lo, hi) in enumerate(X_PARTS)]
        go0_cp = [rows_cp(go_hbm.at[0], go_s.at[0], lo, hi - lo, ("go0", k)) for k, (lo, hi) in enumerate(GO_PARTS)]
        x1_cp = rows_cp(x_hbm.at[1], x_s.at[1], 0, T, "x1")
        go1_cp = rows_cp(go_hbm.at[1], go_s.at[1], 0, TF * U, "go1")
        w1_cp = [cp(w1_hbm, w1_s, "w1")]
        w_cp = [cp(w2_hbm, w2_s, "w2"), cp(wf_hbm, wf_s, "wf"), cp(wg_hbm, wg_s, "wg"), cp(wo_hbm, wo_s, "wo"),
                cp(g_hbm, g_s, "g")]
        out_cp = [[cp(out_s.at[b], out_hbm.at[b], ("out", b))] for b in range(B)]
        dx_cp = [rows_cp(dx_s.at[b], dx_hbm.at[b], 0, T, ("dx", b)) for b in range(B)]
        dw1_cp = [cp(o_dw1.at[pl.ds(k * D, D)], dw1_hbm.at[pl.ds(k * D, D)], ("dw1", k)) for k in range(3)]
        dw2_cp = [cp(o_dw2, dw2_hbm, "dw2")]
        dwf_cp = [cp(o_dwf, dwf_hbm, "dwf")]
        dwg_cp = [cp(o_dwg, dwg_hbm, "dwg")]
        dwo_cp = [cp(o_dwo, dwo_hbm, "dwo")]
        dg_cp = [cp(o_dg, dg_hbm, "dg")]

        start(w1_cp)
        for cs in x0_cp:
            start(cs)
        start(w_cp)
        for cs in go0_cp:
            start(cs)
        start(x1_cp)
        start(go1_cp)
        for b in range(B):
            x_s[b, T:XP, :] = jnp.zeros((XP - T, D), BF16)
        wait(w1_cp)
        wait(x0_cp[0])
        _st(w1_p, 0, w1_s[...])
        _st(ws1_s, 0, _bf(w1_s[0:D, :].astype(F32) + w1_s[2 * D:3 * D, :].astype(F32)))
        zeros8 = jnp.zeros((8, D), F32)

        x_waits = {lo // 4: k for k, (lo, hi) in enumerate(X_PARTS) if k > 0}
        go_waits = {lo // U: k for k, (lo, hi) in enumerate(GO_PARTS)}
        c1_chunks = _chunks(NR, RC1)
        q2 = _chunks(NQ, QC2)
        qb = _chunks(NQ, QCB)
        jchunks = _chunks(TF, CT)

        def conv1_fwd_tasks(b):
            carry = {"x3": zeros8, "h3": zeros8}

            def task(r0, rc):
                if b == 0 and r0 in x_waits:
                    wait(x0_cp[x_waits[r0]])
                xw = _words(x_s[b, 4 * r0:4 * (r0 + rc), :])
                we = _words(_lo16(xw))
                wo_ = _words(_hi16(xw))
                X1, X3 = _lo(wo_), _hi(wo_)
                X3s = _shift_down(X3, carry["x3"])
                carry["x3"] = X3[rc - 8:]
                xa = jnp.concatenate([_bf(X3s - X1), _lo16(we)], axis=1)
                xb = jnp.concatenate([_hi16(we), _bf(X3 - X1)], axis=1)
                x1 = _lo16(wo_)
                _st(xa_s.at[b], r0, xa)
                _st(xb_s.at[b], r0, xb)
                _st(x1_s.at[b], r0, x1)
                m2 = _nn(x1, _ld(ws1_s, 0, D))
                He, gpe = _gelu_and_grad(_nn(xa, _ld(w1_p, 0, 2 * D)) + m2)
                Ho, gpo = _gelu_and_grad(_nn(xb, _ld(w1_p, D, 3 * D)) + m2)
                _st(gpe_s, r0, _bf(gpe))
                _st(gpo_s, r0, _bf(gpo))
                q0, qc = r0 // 2, rc // 2
                hew = _words(_bf(He))
                how = _words(_bf(Ho))
                H1, H3 = _lo(how), _hi(how)
                H3s = _shift_down(H3, carry["h3"])
                carry["h3"] = H3[qc - 8:]
                _st(ha_s, q0, jnp.concatenate([_bf(H3s - H1), _lo16(hew)], axis=1))
                _st(hb_s, q0, jnp.concatenate([_hi16(hew), _bf(H3 - H1)], axis=1))
                _st(h1_s, q0, _lo16(how))

            return [functools.partial(task, r0, rc) for (r0, rc) in c1_chunks]

        def acc_store(b, acc, stage, k, part):
            rows = slice(k * D, (k + 1) * D)
            if b == 0 and NB > 1:
                acc[rows, :] = part
            elif b == 0:
                stage[rows, :] = _bf(part)
            else:
                stage[rows, :] = _bf(acc[rows, :] + part)

        def dw_tasks(b):
            last = b == NB - 1
            st = {}

            def t2a():
                de, do = de_s[0:NQ, :], do_s[0:NQ, :]
                st["p2"] = _tn(_ld(h1_s, 0, NQ), _bf(de + do))
                st["pa"] = _tn(_ld(ha_s, 0, NQ), _bf(de))
                acc_store(b, a_dw2, o_dw2, 0, st["pa"][0:D] + st["p2"])

            def t2b():
                pb = _tn(_ld(hb_s, 0, NQ), _bf(do_s[0:NQ, :]))
                acc_store(b, a_dw2, o_dw2, 1, st["pa"][D:2 * D] + pb[0:D])
                acc_store(b, a_dw2, o_dw2, 2, st["p2"] + pb[D:2 * D])
                if last:
                    start(dw2_cp)

            def t1a():
                st["p2"] = _tn(_ld(x1_s.at[b], 0, NR), _ld(ds_s, 0, NR))

            def t1b():
                pa = _tn(_ld(xa_s.at[b], 0, NR, 0, H), _ld(da_s, 0, NR))
                acc_store(b, a_dw1, o_dw1, 0, pa + st["p2"])
                if last:
                    start(dw1_cp[0:1])

            def t1c():
                x02 = jnp.concatenate([_ld(xa_s.at[b], 0, NR, H, 2 * H), _ld(xb_s.at[b], 0, NR, 0, H)], axis=0)
                dab = jnp.concatenate([_ld(da_s, 0, NR), _ld(db_s, 0, NR)], axis=0)
                acc_store(b, a_dw1, o_dw1, 1, _tn(x02, dab))
                if last:
                    start(dw1_cp[1:2])

            def t1d():
                pb = _tn(_ld(xb_s.at[b], 0, NR, H, 2 * H), _ld(db_s, 0, NR))
                acc_store(b, a_dw1, o_dw1, 2, st["p2"] + pb)
                if last:
                    start(dw1_cp[2:3])

            return [t2a, t2b, t1a, t1b, t1c, t1d]

        for t in conv1_fwd_tasks(0):
            t()

        for b in range(NB):
            if b == 0:
                wait(w_cp)
                _st(w2_p, 0, w2_s[...])
                _st(wf_p, 0, wf_s[...])
                _st(wg_p, 0, wg_s[...])
                _st(wo_p, 0, wo_s[...])
                _st(ws2_s, 0, _bf(w2_s[0:D, :].astype(F32) + w2_s[2 * D:3 * D, :].astype(F32)))
            ge = _nn(g_s[b], _ld(wg_p, 0, D))

            for (q0, qc) in q2:
                m2 = _nn(_ld(h1_s, q0, q0 + qc), _ld(ws2_s, 0, D))
                Fe, gpa = _gelu_and_grad(_nn(_ld(ha_s, q0, q0 + qc), _ld(w2_p, 0, 2 * D)) + m2)
                Fo, gpb = _gelu_and_grad(_nn(_ld(hb_s, q0, q0 + qc), _ld(w2_p, D, 3 * D)) + m2)
                gp2_s[0, q0:q0 + qc, :] = gpa
                gp2_s[1, q0:q0 + qc, :] = gpb
                _st(fb_s.at[0], q0, _bf(Fe))
                _st(fb_s.at[1], q0, _bf(Fo))

            def go_wait(t0):
                if b == 0 and t0 in go_waits:
                    wait(go0_cp[go_waits[t0]])

            def do_fe(c):
                t0, ct = jchunks[c]
                q0, qn = t0 // 2, -(-(ct // 2) // 8) * 8
                fbc = jnp.concatenate([_ld(fb_s.at[0], q0, q0 + qn), _ld(fb_s.at[1], q0, q0 + qn)], axis=0)
                fe = _nn(fbc, _ld(wf_p, 0, D))
                fe_s[0, q0:q0 + qn, :] = fe[:qn]
                fe_s[1, q0:q0 + qn, :] = fe[qn:]

            def do_t(c):
                t0, ct = jchunks[c]
                js = []
                for t in range(t0, t0 + ct):
                    row = jnp.broadcast_to(fe_s[t % 2, pl.ds(t // 2, 1), :], (U, D))
                    js.append(jnp.tanh(row + ge))
                j = jnp.concatenate(js, axis=0)
                return _bf(j), 1.0 - j * j

            def do_dj(c):
                t0, ct = jchunks[c]
                go_wait(t0)
                return _nt(go_s[b, U * t0:U * (t0 + ct), :], _ld(wo_p, 0, D))

            def do_v(c, dj, s):
                t0, ct = jchunks[c]
                dp = dj * s
                dps = [dp[U * i:U * (i + 1)] for i in range(ct)]
                for i0 in range(0, ct, 16):
                    for p in range(2):
                        v = [dps[i] if i < ct else zeros8 for i in range(i0 + p, i0 + 16, 2)]
                        q = (t0 + i0) // 2
                        dfe_s[p, q:q + 8, :] = _rowsum8(v)
                return _tree_sum(dps)

            def do_s3(c, jb):
                t0, ct = jchunks[c]
                out_s[b, U * t0:U * (t0 + ct), :] = _bf(_nn(jb, _ld(wo_p, 0, D)))
                part = _tn(jb, go_s[b, U * t0:U * (t0 + ct), :])
                if b == 0 and c == 0:
                    a_dwo[...] = part
                else:
                    a_dwo[...] += part

            n = len(jchunks)
            do_fe(0)
            jb, s = do_t(0)
            dj = do_dj(0)
            if n > 1:
                do_fe(1)
            dge = None
            for c in range(n):
                part = do_v(c, dj, s)
                dge = part if dge is None else dge + part
                jc = jb
                if c + 1 < n:
                    jb, s = do_t(c + 1)
                do_s3(c, jc)
                if c + 1 < n:
                    dj = do_dj(c + 1)
                if c + 2 < n:
                    do_fe(c + 2)
            start(out_cp[b])
            if b == 0 and NB > 1:
                wait(x1_cp)
                wait(go1_cp)
            if b == NB - 1:
                o_dwo[...] = _bf(a_dwo[...])
                start(dwo_cp)

            dgeb = _bf(dge)
            o_dg[b] = _bf(_nt(dgeb, _ld(wg_p, 0, D)))
            dwg_part = _tn(g_s[b], dgeb)
            if b == 0:
                a_dwg[...] = dwg_part
            if b == NB - 1:
                o_dwg[...] = _bf(a_dwg[...] + dwg_part) if b > 0 else _bf(dwg_part)
                start(dwg_cp)
                start(dg_cp)

            for (q0, qc) in qb:
                dfeb = _bf(jnp.concatenate([dfe_s[0, q0:q0 + qc, :], dfe_s[1, q0:q0 + qc, :]], axis=0))
                df = _nt(dfeb, _ld(wf_p, 0, D))
                de_s[q0:q0 + qc, :] = df[:qc] * gp2_s[0, q0:q0 + qc, :]
                do_s[q0:q0 + qc, :] = df[qc:] * gp2_s[1, q0:q0 + qc, :]
                fbc = jnp.concatenate([_ld(fb_s.at[0], q0, q0 + qc), _ld(fb_s.at[1], q0, q0 + qc)], axis=0)
                part = _tn(fbc, dfeb)
                if b == 0 and q0 == 0:
                    a_dwf[...] = part
                else:
                    a_dwf[...] += part
            if b == NB - 1:
                o_dwf[...] = _bf(a_dwf[...])
                start(dwf_cp)

            def do_dh(ci):
                q0, qc = qb[ci]
                de = de_s[q0:q0 + qc, :]
                do = do_s[q0:q0 + qc, :]
                nxt = de_s[q0 + qc:q0 + qc + 8, :] if ci + 1 < len(qb) else zeros8
                des = _shift_up(de, nxt)
                dob = _bf(do)
                n2 = _nt(dob, _ld(ws2_s, 0, D))
                dH1 = _nt(_bf(de - do), _ld(w2_p, 2 * D, 3 * D)) + n2
                dH3 = _nt(_bf(des - do), _ld(w2_p, 0, D)) + n2
                dH0 = _nt(_bf(de), _ld(w2_p, D, 2 * D))
                dH2 = _nt(dob, _ld(w2_p, D, 2 * D))
                r0, rc = 2 * q0, 2 * qc
                gew = _ldw(gpe_s, r0, r0 + rc)
                gow = _ldw(gpo_s, r0, r0 + rc)
                return (dH0 * _lo(gew), dH1 * _lo(gow), dH2 * _hi(gew), dH3 * _hi(gow))

            def do_dx(ci, d, nxt):
                q0, qc = qb[ci]
                d0, d1, d2, d3 = d
                d0s = _shift_up(d0, nxt)
                r0, rc = 2 * q0, 2 * qc
                A = _il(d0, d2)
                Bo = _il(d1, d3)
                N1 = _il(d0 - d1, d2 - d3)
                N3 = _il(d2 - d1, d0s - d3)
                _st(da_s, r0, A)
                _st(db_s, r0, Bo)
                _st(ds_s, r0, _il(d0 + d1, d2 + d3))
                n2 = _nt(Bo, _ld(ws1_s, 0, D))
                dX1 = _nt(N1, _ld(w1_p, 2 * D, 3 * D)) + n2
                dX3 = _nt(N3, _ld(w1_p, 0, D)) + n2
                dhp = _il(A.astype(F32), Bo.astype(F32))
                P = _nt(dhp, _ld(w1_p, D, 2 * D))
                Q = _il(dX1, dX3).astype(F32)
                dx_s[b, 4 * r0:4 * (r0 + rc), :] = _il(P, Q)

            d_cur = do_dh(0)
            for ci in range(len(qb)):
                d_nxt = do_dh(ci + 1) if ci + 1 < len(qb) else None
                do_dx(ci, d_cur, d_nxt[0][0:8] if d_nxt is not None else zeros8)
                d_cur = d_nxt
            start(dx_cp[b])

            dwt = dw_tasks(b)
            if b + 1 < NB:
                c1t = conv1_fwd_tasks(b + 1)
                order = dwt[0:2]
                rest = dwt[2:]
                k = 0
                for t in c1t:
                    if k < len(rest):
                        order.append(rest[k]); k += 1
                    order.append(t)
                order += rest[k:]
                for t in order:
                    t()
            else:
                for t in dwt:
                    t()

        for b in range(NB):
            wait(out_cp[b])
            wait(dx_cp[b])
        if NB == 1:
            wait(x1_cp)
            wait(go1_cp)
        for cs in (dwo_cp, dwg_cp, dg_cp, dwf_cp, dw2_cp, dw1_cp):
            wait(cs)

    bufs = dict(TF=TF, NQ=NQ, NQP=NQP, NR=NR, XP=XP, H=H)
    return kernel, bufs


def _run(x, w1, w2, g, w_f, w_g, w_o, grad_out, NB=2, RC1=(192, 320, 256, 240), QC2=256, QCB=128, CT=32,
        X_PARTS=((0, 768), (768, 2048), (2048, 4000)), GO_PARTS=((0, 3072), (3072, 8000))):
    B, T, D = x.shape
    U = g.shape[1]
    TF = T // 4
    go = grad_out.reshape(B, TF * U, D)
    w1c = w1.reshape(3 * D, D)
    w2c = w2.reshape(3 * D, D)
    kernel, s = make_kernel(B, T, D, U, NB, RC1, QC2, QCB, CT, X_PARTS, GO_PARTS)
    NQ, NQP, NR, XP, H = s["NQ"], s["NQP"], s["NR"], s["XP"], s["H"]
    any_spec = pl.BlockSpec(memory_space=pl.ANY)
    sds = lambda sh: jax.ShapeDtypeStruct(sh, BF16)
    out_shape = [sds((B, TF * U, D)), sds((B, T, D)), sds((3 * D, D)), sds((3 * D, D)),
                 sds((B, U, D)), sds((D, D)), sds((D, D)), sds((D, D))]
    V = pltpu.VMEM
    P = lambda ncol, rows: (ncol, rows // 2, L)
    scratch = [
        V((B, XP, D), BF16), V((B, TF * U, D), BF16), V((B, TF * U, D), BF16), V((B, XP, D), BF16),
        V((3 * D, D), BF16), V((3 * D, D), BF16), V((D, D), BF16), V((D, D), BF16), V((D, D), BF16),
        V((B, U, D), BF16),
        V(P(H, 3 * D), U32), V(P(H, 3 * D), U32), V(P(H, D), U32), V(P(H, D), U32), V(P(H, D), U32),
        V(P(H, D), U32), V(P(H, D), U32),
        V((3 * D, D), BF16), V((3 * D, D), BF16), V((D, D), BF16), V((D, D), BF16), V((D, D), BF16), V((B, U, D), BF16),
        V((3 * D, D), F32), V((3 * D, D), F32), V((D, D), F32), V((D, D), F32), V((D, D), F32),
        V((B,) + P(2 * H, NR), U32), V((B,) + P(2 * H, NR), U32), V((B,) + P(H, NR), U32),
        V(P(H, NR), U32), V(P(H, NR), U32),
        V(P(2 * H, NQP), U32), V(P(2 * H, NQP), U32), V(P(H, NQP), U32),
        V((2, NQ, D), F32), V((2,) + P(H, NQP), U32), V((2, NQ, D), F32), V((2, NQ, D), F32),
        V((NQ, D), F32), V((NQ, D), F32), V(P(H, NR), U32), V(P(H, NR), U32), V(P(H, NR), U32),
        pltpu.SemaphoreType.DMA((40,)),
    ]
    outs = pl.pallas_call(
        kernel,
        in_specs=[any_spec] * 8, out_specs=[any_spec] * 8, out_shape=out_shape,
        scratch_shapes=scratch,
        compiler_params=pltpu.CompilerParams(vmem_limit_bytes=110 * 2**20),
    )(x, go, g, w1c, w2c, w_f, w_g, w_o)
    out, dx, dw1, dw2, dg, dwf, dwg, dwo = outs
    return (out.reshape(B, TF, U, D), dx, dw1.reshape(3, D, D), dw2.reshape(3, D, D), dg, dwf, dwg, dwo)


@jax.jit
def pallas_standalone__seq2seq_rnn_t_joint__speech_kernel(
    x: jax.Array,
    w1: jax.Array,
    w2: jax.Array,
    g: jax.Array,
    w_f: jax.Array,
    w_g: jax.Array,
    w_o: jax.Array,
    grad_out: jax.Array,
):
    return _run(x, w1, w2, g, w_f, w_g, w_o, grad_out)
```

```python
import functools

import jax
import jax.numpy as jnp
from jax.experimental import pallas as pl
from jax.experimental.pallas import tpu as pltpu

F32 = jnp.float32
BF16 = jnp.bfloat16
U32 = jnp.uint32
L = 128

_C = 0.7978845608028654
_K = 0.044715


def _gelu_and_grad(x):
    x2 = x * x
    t = jnp.tanh(x * (_C + (_C * _K) * x2))
    p = 0.5 + 0.5 * t
    g = x * p
    gp = p + g * (1.0 - p) * (2.0 * _C + (6.0 * _C * _K) * x2)
    return g, gp


def _bf(a):
    return a.astype(BF16)


def _words(a_bf16):
    return pltpu.bitcast(a_bf16, U32)


def _unwords(w):
    return pltpu.bitcast(w, BF16)


def _lo(w):
    return pltpu.bitcast(w << 16, F32)


def _hi(w):
    return pltpu.bitcast(w & jnp.uint32(0xFFFF0000), F32)


def _il(a, b):
    return _unwords(pltpu.pack_elementwise([a, b], packed_dtype=BF16))


def _nn(a, b):
    return jnp.dot(a, b, preferred_element_type=F32)


def _nt(a, b):
    return jax.lax.dot_general(a, b, (((1,), (1,)), ((), ())), preferred_element_type=F32)


def _tn(a, b):
    return jax.lax.dot_general(a, b, (((0,), (0,)), ((), ())), preferred_element_type=F32)


def _shift_up(a, next8):
    n = a.shape[0]
    return pltpu.roll(jnp.concatenate([a, next8], axis=0), n + 7, 0)[:n]


def _ld(ref, r0, r1, c0=0, c1=None):
    c1 = ref.shape[0] if c1 is None else c1
    parts = [_unwords(ref[c, r0 // 2:r1 // 2, :]) for c in range(c0, c1)]
    return parts[0] if len(parts) == 1 else jnp.concatenate(parts, axis=1)


def _st(ref, r0, val):
    w = _words(val)
    for c in range(val.shape[1] // L):
        ref[c, r0 // 2:(r0 + val.shape[0]) // 2, :] = w[:, c * L:(c + 1) * L]


def _st32(ref, r0, val):
    for c in range(val.shape[1] // L):
        ref[c, r0:r0 + val.shape[0], :] = val[:, c * L:(c + 1) * L]


def _lds(ref, start, n, stride):
    return jnp.concatenate([ref[c, pl.ds(start, n, stride=stride), :] for c in range(ref.shape[0])], axis=1)


def _blocks(a, h):
    c = a.shape[1] // 2
    return a[:h, :c], a[:h, c:], a[h:, :c], a[h:, c:]


def _strassen_out(m1, m2, m3, m4, m5, m6, m7):
    return m1 + m4 - m5 + m7, m3 + m5, m2 + m4, m1 - m2 + m3 + m6


def _rowsum8(v):
    s = jax.lax.broadcasted_iota(jnp.int32, v[0].shape, 0)

    def comb(a, b, m, k):
        return jnp.where(m, a, b) + pltpu.roll(jnp.where(m, b, a), 8 - k, 0)

    m4 = lambda j: ((s + (8 - j)) & 4) == 0
    m2 = lambda j: ((s + (8 - j)) & 2) == 0
    ab = comb(v[0], v[4], m4(0), 4)
    cd = comb(v[2], v[6], m4(2), 4)
    ef = comb(v[1], v[5], m4(1), 4)
    gh = comb(v[3], v[7], m4(3), 4)
    return comb(comb(ab, cd, m2(0), 2), comb(ef, gh, m2(1), 2), (s & 1) == 0, 1)


def _tree_sum(v):
    v = list(v)
    while len(v) > 1:
        v = [v[i] + v[i + 1] if i + 1 < len(v) else v[i] for i in range(0, len(v), 2)]
    return v[0]


def _chunks(total, size):
    sizes = list(size) if isinstance(size, (tuple, list)) else [min(size, total - s) for s in range(0, total, size)]
    assert sum(sizes) == total, (size, total)
    return [(sum(sizes[:i]), n) for i, n in enumerate(sizes)]


def _make_kernel(B, T, D, U, RC1, QC2, QCB, CT, FE, X_PARTS, FIFO, ORDER):
    TF = T // 4
    NQ = -(-(TF // 2) // 8) * 8
    NR = 2 * NQ
    XP = 4 * NR
    H = D // L
    PAD = 8
    J0 = U * CT

    sem_ids = {}

    def sid(name, n=1):
        if name not in sem_ids:
            sem_ids[name] = (sum(k for _, k in sem_ids.values()), n)
        return sem_ids[name][0]

    def kernel(x_hbm, go_hbm, g_hbm, w1_hbm, w2_hbm, wf_hbm, wg_hbm, wo_hbm,
               out_hbm, dx_hbm, dw1_hbm, dw2_hbm, dg_hbm, dwf_hbm, dwg_hbm, dwo_hbm,
               x_s, go_s, out_s, dx_s, w1_s, w2_s, wf_s, wg_s, wo_s, g_s,
               w1_p, w2_p, wf_p, wg_p, wt_p, wn_p, ws1_p, ws2_p,
               o_dw1, o_dw2, o_dwf, o_dwg, o_dwo, o_dg,
               a_dwf, a_dwg, a_dwo,
               xw_s, xa_s, xb_s, x1_s, he_s, ho_s, gpe_s, gpo_s, ha_s, hb_s, h1_s, gp2_s, f_s,
               ge_s, fe_s, jb0_s, s0_s, dfe_s, de_s, do_s, da_s, db_s, ds_s,
               sems):
        def cp(src, dst, name):
            return pltpu.make_async_copy(src, dst, sems.at[sid(name)])

        def cp_b(src, dst, name, b):
            return pltpu.make_async_copy(src, dst, sems.at[sid(name, B) + b])

        def start(cs):
            for c in cs:
                c.start()

        def wait(cs):
            for c in cs:
                c.wait()

        in_cp = {"w1": cp(w1_hbm, w1_s, "w1"), "w2": cp(w2_hbm, w2_s, "w2"), "wf": cp(wf_hbm, wf_s, "wf"),
                 "wg": cp(wg_hbm, wg_s, "wg"), "wo": cp(wo_hbm, wo_s, "wo"), "g": cp(g_hbm, g_s, "g")}
        for name, (b, lo, hi) in X_PARTS.items():
            in_cp[name] = cp(x_hbm.at[b, pl.ds(lo, hi - lo)], x_s.at[b, pl.ds(lo, hi - lo)], name)
        go_cp = lambda b: cp_b(go_hbm.at[b], go_s.at[b], "go", b)
        out_cp = lambda b: cp_b(out_s.at[b], out_hbm.at[b], "out", b)
        dx_cp = lambda b: cp_b(dx_s.at[b, pl.ds(0, T)], dx_hbm.at[b], "dx", b)
        dw1_rows = [(0, D), (D, D)] + [(2 * D + c * L, L) for c in range(H)]
        dw1_cp = [cp(o_dw1.at[pl.ds(lo, n)], dw1_hbm.at[pl.ds(lo, n)], ("dw1", lo)) for lo, n in dw1_rows]
        dw2_cp = [cp(o_dw2, dw2_hbm, "dw2")]
        small_cp = [cp(o_dwo, dwo_hbm, "dwo"), cp(o_dwf, dwf_hbm, "dwf"), cp(o_dwg, dwg_hbm, "dwg"),
                    cp(o_dg, dg_hbm, "dg")]

        start([in_cp[name] for name in FIFO])
        for b in range(B):
            go_cp(b).start()
        for b in range(B):
            x_s[b, T:XP, :] = jnp.zeros((XP - T, D), BF16)
            for c in range(H):
                xw_s[b, c, 0:PAD, :] = jnp.zeros((PAD, L), U32)
                ho_s[b, c, 0:PAD, :] = jnp.zeros((PAD, L), F32)
        for acc in (a_dwf, a_dwg, a_dwo):
            acc[...] = jnp.zeros(acc.shape, F32)
        wait([in_cp["w1"]])
        _st(w1_p, 0, w1_s[...])
        _st(ws1_p, 0, _bf(w1_s[0:D, :].astype(F32) + w1_s[2 * D:3 * D, :].astype(F32)))
        zeros8 = jnp.zeros((8, D), F32)

        c1_chunks = [_chunks(NR, RC1[b]) for b in range(B)]
        q2 = _chunks(NQ, QC2)
        qb = _chunks(NQ, QCB)
        jchunks = _chunks(TF, CT)

        def prepare_w2():
            _st(w2_p, 0, w2_s[...])
            _st(ws2_p, 0, _bf(w2_s[0:D, :].astype(F32) + w2_s[2 * D:3 * D, :].astype(F32)))

        def prepare_joint_weights():
            _st(wf_p, 0, wf_s[...])
            _st(wg_p, 0, wg_s[...])
            w11, w12, w21, w22 = _blocks(wo_s[...].astype(F32), D // 2)
            for i, v in enumerate((w11 + w22, w11, w21 - w22, w12 - w11, w22, w11 + w21, w12 + w22)):
                wt_p[i] = _words(_bf(v))
            for i, v in enumerate((w11 + w22, w12 + w22, w11, w22, w11 + w21, w12 - w11, w21 - w22)):
                wn_p[i] = _words(_bf(v))

        def conv1_fwd(b, k):
            r0, rc = c1_chunks[b][k]
            xw = xw_s.at[b]
            _st32(xw, PAD + 2 * r0, _words(x_s[b, 4 * r0:4 * (r0 + rc), :]))
            q0, qc = r0 // 2, rc // 2
            z = [_lds(xw, PAD + 4 * q0 + j, qc, 4) for j in range(4)]
            y0, y1, y2, y3, y4, y5, y6, y7 = [f(w) for w in z for f in (_lo, _hi)]
            y7s = _hi(_lds(xw, PAD + 4 * q0 - 1, qc, 4))
            xa = jnp.concatenate([_il(y7s - y1, y3 - y5), _il(y0, y4)], axis=1)
            xb = jnp.concatenate([_il(y2, y6), _il(y3 - y1, y7 - y5)], axis=1)
            x1 = _il(y1, y5)
            _st(xa_s.at[b], r0, xa)
            _st(xb_s.at[b], r0, xb)
            _st(x1_s.at[b], r0, x1)
            m2 = _nn(x1, _ld(ws1_p, 0, D))
            hpre = _nn(xa, _ld(w1_p, 0, 2 * D)) + m2
            ho, gpo = _gelu_and_grad(_nn(xb, _ld(w1_p, D, 3 * D)) + m2)
            he, gpe = _gelu_and_grad(hpre)
            _st32(he_s.at[b], r0, he)
            _st32(ho_s.at[b], PAD + r0, ho)
            _st32(gpe_s.at[b], r0, gpe)
            _st32(gpo_s.at[b], r0, gpo)

        def conv2_fwd(b, k):
            q0, qc = q2[k]
            pc = qc // 2
            he, ho = he_s.at[b], ho_s.at[b]
            g0, g1, g2, g3 = [_lds(he, 2 * q0 + j, pc, 4) for j in range(4)]
            o0, o1, o2, o3 = [_lds(ho, PAD + 2 * q0 + j, pc, 4) for j in range(4)]
            o3s = _lds(ho, PAD + 2 * q0 - 1, pc, 4)
            ha = jnp.concatenate([_il(o3s - o0, o1 - o2), _il(g0, g2)], axis=1)
            hb = jnp.concatenate([_il(g1, g3), _il(o1 - o0, o3 - o2)], axis=1)
            h1 = _il(o0, o2)
            _st(ha_s.at[b], q0, ha)
            _st(hb_s.at[b], q0, hb)
            _st(h1_s.at[b], q0, h1)
            m2 = _nn(h1, _ld(ws2_p, 0, D))
            fe, gpa = _gelu_and_grad(_nn(ha, _ld(w2_p, 0, 2 * D)) + m2)
            fo, gpb = _gelu_and_grad(_nn(hb, _ld(w2_p, D, 3 * D)) + m2)
            gp2_s[b, 0, q0:q0 + qc, :] = gpa
            gp2_s[b, 1, q0:q0 + qc, :] = gpb
            f_s[b, 0, q0:q0 + qc, :] = fe
            f_s[b, 1, q0:q0 + qc, :] = fo

        def do_fe(b, t0, t1):
            q0, qn = t0 // 2, -(-((t1 - t0) // 2) // 8) * 8
            fb = _bf(jnp.concatenate([f_s[b, 0, q0:q0 + qn, :], f_s[b, 1, q0:q0 + qn, :]], axis=0))
            fe = _nn(fb, _ld(wf_p, 0, D))
            fe_s[b, 0, q0:q0 + qn, :] = fe[:qn]
            fe_s[b, 1, q0:q0 + qn, :] = fe[qn:]

        def do_t(b, c):
            t0, ct = jchunks[c]
            ge = ge_s[b]
            js = [jnp.tanh(jnp.broadcast_to(fe_s[b, t % 2, pl.ds(t // 2, 1), :], (U, D)) + ge)
                  for t in range(t0, t0 + ct)]
            j = jnp.concatenate(js, axis=0)
            j11, j12, j21, j22 = _blocks(j, U * ct // 2)
            jb = [_bf(v) for v in (j11 + j22, j11, j21 - j22, j12 - j11, j22, j11 + j21, j12 + j22)]
            return jb, 1.0 - j * j

        def joint_head(b):
            ge_s[b] = _nn(g_s[b], _ld(wg_p, 0, D))
            do_fe(b, 0, FE)
            jb, s = do_t(b, 0)
            for i in range(7):
                jb0_s[b, i] = _words(jb[i])
            s0_s[b] = s

        for task in ORDER:
            if task[0] == "w":
                wait([in_cp[name] for name in task[1:]])
            elif task[0] == "c1":
                conv1_fwd(*task[1:])
            elif task[0] == "c2":
                conv2_fwd(*task[1:])
            elif task[0] == "head":
                joint_head(task[1])
            elif task[0] == "pw2":
                prepare_w2()
            else:
                prepare_joint_weights()

        def batch_step(b, carry):
            go_cp(b).wait()

            wt = lambda i: _unwords(wt_p[i])
            wn = lambda i: _unwords(wn_p[i])

            def do_dj(c):
                t0, ct = jchunks[c]
                h = U * ct // 2
                gt = go_s[b, U * t0:U * t0 + h, :]
                gb = go_s[b, U * t0 + h:U * t0 + 2 * h, :]
                g11, g12, g21, g22 = gt[:, :L], gt[:, L:], gb[:, :L], gb[:, L:]
                f11, f12, f21, f22 = [v.astype(F32) for v in (g11, g12, g21, g22)]
                ga = [_bf(f11 + f22), _bf(f21 + f22), g11, g22, _bf(f11 + f12), _bf(f21 - f11), _bf(f12 - f22)]
                n = {i: _nt(ga[i], wt(i)) for i in (0, 3, 4, 6, 1, 2, 5)}
                d11, d12, d21, d22 = _strassen_out(*[n[i] for i in range(7)])
                dj = jnp.concatenate([jnp.concatenate([d11, d12], axis=1), jnp.concatenate([d21, d22], axis=1)], axis=0)
                return dj, ga

            def do_v(c, dj, s):
                t0, ct = jchunks[c]
                dp = dj * s
                dps = [dp[U * i:U * (i + 1)] for i in range(ct)]
                for i0 in range(0, ct, 16):
                    for p in range(2):
                        v = [dps[i] if i < ct else zeros8 for i in range(i0 + p, i0 + 16, 2)]
                        q = (t0 + i0) // 2
                        dfe_s[p, q:q + 8, :] = _rowsum8(v)
                return _tree_sum(dps)

            def do_out(c, jb):
                t0, ct = jchunks[c]
                h = U * ct // 2
                m = {i: _nn(jb[i], wn(i)) for i in (0, 3, 4, 6, 1, 2, 5)}
                o11, o21, o12, o22 = _strassen_out(*[m[i] for i in range(7)])
                out_s[b, U * t0:U * t0 + h, :] = _bf(jnp.concatenate([o11, o12], axis=1))
                out_s[b, U * t0 + h:U * t0 + 2 * h, :] = _bf(jnp.concatenate([o21, o22], axis=1))

            def do_dwo(jb, ga):
                pairs = ((0, 0), (6, 2), (1, 6), (4, 5), (5, 3), (3, 4), (2, 1))
                for i in (4, 0, 2, 6, 1, 5, 3):
                    a_dwo[i] += _tn(ga[pairs[i][1]], jb[pairs[i][0]])

            n = len(jchunks)
            fe_done = [FE]

            def need_fe(t1):
                while fe_done[0] < min(t1, TF):
                    t0 = fe_done[0]
                    fe_done[0] = min(t0 + FE, TF)
                    do_fe(b, t0, fe_done[0])

            jb, s = [_unwords(jb0_s[b, i]) for i in range(7)], s0_s[b]
            dj, ga = do_dj(0)
            dge = None
            prev = None
            for c in range(n):
                part = do_v(c, dj, s)
                dge = part if dge is None else dge + part
                cur = (jb, ga)
                do_out(c, jb)
                if c + 1 < n:
                    need_fe(jchunks[c + 1][0] + jchunks[c + 1][1])
                    jb, s = do_t(b, c + 1)
                if prev is not None:
                    do_dwo(*prev)
                prev = cur
                if c + 1 < n:
                    dj, ga = do_dj(c + 1)
            do_dwo(*prev)
            out_cp(b).start()

            dgeb = _bf(dge)
            o_dg[b] = _bf(_nt(dgeb, _ld(wg_p, 0, D)))
            dwg = a_dwg[...] + _tn(g_s[b], dgeb)
            a_dwg[...] = dwg
            o_dwg[...] = _bf(dwg)
            p1, p2, p3, p4, p5, p6, p7 = [a_dwo[i] for i in range(7)]
            o_dwo[0:L, :] = _bf(jnp.concatenate([(p1 + p4 - p5 + p7).T, (p3 + p5).T], axis=1))
            o_dwo[L:D, :] = _bf(jnp.concatenate([(p2 + p4).T, (p1 - p2 + p3 + p6).T], axis=1))

            for (q0, qc) in qb:
                dfeb = _bf(jnp.concatenate([dfe_s[0, q0:q0 + qc, :], dfe_s[1, q0:q0 + qc, :]], axis=0))
                df = _nt(dfeb, _ld(wf_p, 0, D))
                de_s[b, q0:q0 + qc, :] = df[:qc] * gp2_s[b, 0, q0:q0 + qc, :]
                do_s[b, q0:q0 + qc, :] = df[qc:] * gp2_s[b, 1, q0:q0 + qc, :]
                fb = _bf(jnp.concatenate([f_s[b, 0, q0:q0 + qc, :], f_s[b, 1, q0:q0 + qc, :]], axis=0))
                a_dwf[...] += _tn(fb, dfeb)
            o_dwf[...] = _bf(a_dwf[...])

            gpe, gpo = gpe_s.at[b], gpo_s.at[b]

            def do_dh(ci):
                q0, qc = qb[ci]
                de = de_s[b, q0:q0 + qc, :]
                do = do_s[b, q0:q0 + qc, :]
                nxt = de_s[b, q0 + qc:q0 + qc + 8, :] if ci + 1 < len(qb) else zeros8
                des = _shift_up(de, nxt)
                dob = _bf(do)
                n2 = _nt(dob, _ld(ws2_p, 0, D))
                dh1 = _nt(_bf(de - do), _ld(w2_p, 2 * D, 3 * D)) + n2
                dh3 = _nt(_bf(des - do), _ld(w2_p, 0, D)) + n2
                dh0 = _nt(_bf(de), _ld(w2_p, D, 2 * D))
                dh2 = _nt(dob, _ld(w2_p, D, 2 * D))
                r0 = 2 * q0
                return (dh0 * _lds(gpe, r0, qc, 2), dh1 * _lds(gpo, r0, qc, 2),
                        dh2 * _lds(gpe, r0 + 1, qc, 2), dh3 * _lds(gpo, r0 + 1, qc, 2))

            def do_dx(ci, d, nxt):
                q0, qc = qb[ci]
                d0, d1, d2, d3 = d
                d0s = _shift_up(d0, nxt)
                r0, rc = 2 * q0, 2 * qc
                a = _il(d0, d2)
                bo = _il(d1, d3)
                _st(da_s.at[b], r0, a)
                _st(db_s.at[b], r0, bo)
                _st(ds_s.at[b], r0, _il(d0 + d1, d2 + d3))
                n2 = _nt(bo, _ld(ws1_p, 0, D))
                dx1 = _nt(_il(d0 - d1, d2 - d3), _ld(w1_p, 2 * D, 3 * D)) + n2
                dx3 = _nt(_il(d2 - d1, d0s - d3), _ld(w1_p, 0, D)) + n2
                dhp = _il(a.astype(F32), bo.astype(F32))
                even = _nt(dhp, _ld(w1_p, D, 2 * D))
                odd = _il(dx1, dx3).astype(F32)
                dx_s[b, 4 * r0:4 * (r0 + rc), :] = _il(even, odd)

            d_cur = do_dh(0)
            for ci in range(len(qb)):
                d_nxt = do_dh(ci + 1) if ci + 1 < len(qb) else None
                do_dx(ci, d_cur, d_nxt[0][0:8] if d_nxt is not None else zeros8)
                d_cur = d_nxt
            dx_cp(b).start()
            return carry

        jax.lax.fori_loop(0, B, batch_step, 0)

        start(small_cp)
        out_cp(0).wait()

        def both(ref, n, c0=0, c1=None):
            return jnp.concatenate([_ld(ref.at[b], 0, n, c0, c1) for b in range(B)], axis=0)

        def both32(fn):
            return _bf(jnp.concatenate([fn(b) for b in range(B)], axis=0))

        p2 = _tn(both(h1_s, NQ), both32(lambda b: de_s[b] + do_s[b]))
        pa = _tn(both(ha_s, NQ), both32(lambda b: de_s[b]))
        o_dw2[0:D, :] = _bf(pa[0:D] + p2)
        pb = _tn(both(hb_s, NQ), both32(lambda b: do_s[b]))
        o_dw2[D:2 * D, :] = _bf(pa[D:2 * D] + pb[0:D])
        o_dw2[2 * D:3 * D, :] = _bf(p2 + pb[D:2 * D])
        start(dw2_cp)
        p2 = _tn(both(x1_s, NR), both(ds_s, NR))
        o_dw1[0:D, :] = _bf(_tn(both(xa_s, NR, 0, H), both(da_s, NR)) + p2)
        start(dw1_cp[0:1])
        x02 = jnp.concatenate([both(xa_s, NR, H, 2 * H), both(xb_s, NR, 0, H)], axis=0)
        dab = jnp.concatenate([both(da_s, NR), both(db_s, NR)], axis=0)
        o_dw1[D:2 * D, :] = _bf(_tn(x02, dab))
        start(dw1_cp[1:2])
        dbb = both(db_s, NR)
        for c in range(H):
            o_dw1[2 * D + c * L:2 * D + (c + 1) * L, :] = _bf(
                p2[c * L:(c + 1) * L] + _tn(both(xb_s, NR, H + c, H + c + 1), dbb))
            start(dw1_cp[2 + c:3 + c])

        out_cp(1).wait()
        for b in range(B):
            dx_cp(b).wait()
        for cs in (small_cp, dw2_cp, dw1_cp):
            wait(cs)

    return kernel, dict(TF=TF, NQ=NQ, NR=NR, XP=XP, H=H, PAD=PAD, J0=J0)


def _run(x, w1, w2, g, w_f, w_g, w_o, grad_out,
        RC1=((192, 320, 256, 240), (256, 256, 256, 240)), QC2=256, QCB=64, CT=32, FE=64,
        X_PARTS=(("xa", (0, 0, 768)), ("xb", (0, 768, 2048)), ("xc", (0, 2048, 4000)),
                 ("xd", (1, 0, 2048)), ("xe", (1, 2048, 4000))),
        FIFO=("w1", "xa", "xb", "xc", "xd", "w2", "wf", "wg", "wo", "g", "xe"),
        ORDER=(("w", "xa"), ("c1", 0, 0), ("w", "xb"), ("c1", 0, 1), ("w", "xc"), ("c1", 0, 2), ("c1", 0, 3),
               ("w", "xd"), ("c1", 1, 0), ("c1", 1, 1), ("w", "xe", "w2", "wf", "wg", "wo", "g"), ("c1", 1, 2),
               ("pw2",), ("c2", 0, 0), ("pj",), ("c1", 1, 3), ("c2", 0, 1), ("head", 0), ("c2", 1, 0),
               ("head", 1), ("c2", 1, 1))):
    B, T, D = x.shape
    U = g.shape[1]
    TF = T // 4
    kernel, s = _make_kernel(B, T, D, U, RC1, QC2, QCB, CT, FE, dict(X_PARTS), FIFO, ORDER)
    NQ, NR, XP, H, PAD, J0 = s["NQ"], s["NR"], s["XP"], s["H"], s["PAD"], s["J0"]
    NQP = -(-NQ // 16) * 16
    any_spec = pl.BlockSpec(memory_space=pl.ANY)
    sds = lambda *sh: jax.ShapeDtypeStruct(sh, BF16)
    out_shape = [sds(B, TF * U, D), sds(B, T, D), sds(3 * D, D), sds(3 * D, D),
                 sds(B, U, D), sds(D, D), sds(D, D), sds(D, D)]
    V = pltpu.VMEM
    P = lambda ncol, rows: (ncol, rows // 2, L)
    scratch = [
        V((B, XP, D), BF16), V((B, TF * U, D), BF16), V((B, TF * U, D), BF16), V((B, XP, D), BF16),
        V((3 * D, D), BF16), V((3 * D, D), BF16), V((D, D), BF16), V((D, D), BF16), V((D, D), BF16),
        V((B, U, D), BF16),
        V(P(H, 3 * D), U32), V(P(H, 3 * D), U32), V(P(H, D), U32), V(P(H, D), U32),
        V(P(7, L), U32), V(P(7, L), U32), V(P(H, D), U32), V(P(H, D), U32),
        V((3 * D, D), BF16), V((3 * D, D), BF16), V((D, D), BF16), V((D, D), BF16), V((D, D), BF16),
        V((B, U, D), BF16),
        V((D, D), F32), V((D, D), F32), V((7, L, L), F32),
        V((B, H, 2 * PAD + 2 * NR, L), U32),
        V((B,) + P(2 * H, NR), U32), V((B,) + P(2 * H, NR), U32), V((B,) + P(H, NR), U32),
        V((B, H, PAD + NR, L), F32), V((B, H, 2 * PAD + NR, L), F32),
        V((B, H, PAD + NR, L), F32), V((B, H, PAD + NR, L), F32),
        V((B,) + P(2 * H, NQP), U32), V((B,) + P(2 * H, NQP), U32), V((B,) + P(H, NQP), U32),
        V((B, 2, NQ, D), F32), V((B, 2, NQ, D), F32),
        V((B, U, D), F32), V((B, 2, NQ, D), F32), V((B,) + P(7, J0 // 2), U32), V((B, J0, D), F32),
        V((2, NQ, D), F32), V((B, NQ, D), F32), V((B, NQ, D), F32),
        V((B,) + P(H, NR), U32), V((B,) + P(H, NR), U32), V((B,) + P(H, NR), U32),
        pltpu.SemaphoreType.DMA((32,)),
    ]
    out, dx, dw1, dw2, dg, dwf, dwg, dwo = pl.pallas_call(
        kernel,
        in_specs=[any_spec] * 8, out_specs=[any_spec] * 8, out_shape=out_shape,
        scratch_shapes=scratch,
        compiler_params=pltpu.CompilerParams(vmem_limit_bytes=110 * 2**20),
    )(x, grad_out.reshape(B, TF * U, D), g, w1.reshape(3 * D, D), w2.reshape(3 * D, D), w_f, w_g, w_o)
    return (out.reshape(B, TF, U, D), dx, dw1.reshape(3, D, D), dw2.reshape(3, D, D), dg, dwf, dwg, dwo)


@jax.jit
def pallas_standalone__seq2seq_rnn_t_joint__speech_kernel(
    x: jax.Array,
    w1: jax.Array,
    w2: jax.Array,
    g: jax.Array,
    w_f: jax.Array,
    w_g: jax.Array,
    w_o: jax.Array,
    grad_out: jax.Array,
):
    return _run(x, w1, w2, g, w_f, w_g, w_o, grad_out)
```
